```python
import os as _os
_os.environ.setdefault("JAX_PLATFORMS", "cpu")
import jax
import jax.numpy as jnp

def _softmax(x, axis=-1):
    return jax.nn.softmax(x, axis=axis)
def _gelu(x):
    return jax.nn.gelu(x, approximate=True)
def _silu(x):
    return jax.nn.silu(x)
def _sigmoid(x):
    return jax.nn.sigmoid(x)
def _layernorm(x, axis=-1, eps=1e-5):
    m = jnp.mean(x, axis=axis, keepdims=True)
    v = jnp.var(x, axis=axis, keepdims=True)
    return (x - m) / jnp.sqrt(v + eps)
def _scatter_add(tgt, idx, src, axis=0):
    return tgt.at[idx].add(src)
def _segment_sum(src, seg, n):
    return jax.ops.segment_sum(src, seg, n)
class _Rng:
    def __init__(self, key):
        self._k = key
    def _next(self):
        self._k, sub = jax.random.split(self._k)
        return sub
    def normal(self, shape):
        return jax.random.normal(self._next(), shape, dtype=jnp.bfloat16)
    def randint(self, lo, hi, shape):
        return jax.random.randint(self._next(), shape, lo, hi, dtype=jnp.int32)
    def uniform(self, shape, lo=0.0, hi=1.0):
        return jax.random.uniform(self._next(), shape, jnp.bfloat16, lo, hi)
    def permutation(self, n):
        return jax.random.permutation(self._next(), n)


kernel_name = 'parallel_sum__ssm_conv_s5__geglu_ffn__prompt'

def setup_inputs():
    _rng = _Rng(jax.random.key(int.from_bytes(__import__("os").urandom(4), "little")))
    _w = (lambda a: (lambda t: t.astype(jnp.bfloat16) if jnp.issubdtype(t.dtype, jnp.floating) else t)(jnp.asarray(a)))
    def _A_setup():
        B, S, D = 1, 2048, 512
        P = D
        Lambda_re = -0.5 * jnp.exp((lambda *s: _rng.normal(s) * 0.8)(P))
        Lambda_im = (lambda *s: _rng.normal(s) * 0.8)(P) * 1.0
        B_re = (lambda *s: _rng.normal(s) * 0.8)(P, D) * (D ** -0.5)
        B_im = (lambda *s: _rng.normal(s) * 0.8)(P, D) * (D ** -0.5)
        C_re = (lambda *s: _rng.normal(s) * 0.8)(D, P) * (P ** -0.5)
        C_im = (lambda *s: _rng.normal(s) * 0.8)(D, P) * (P ** -0.5)
        log_dt = (lambda *s: _rng.normal(s) * 0.8)(P) * 0.3 - 2.0
        Dskip = (lambda *s: _rng.normal(s) * 0.8)(D)
        return {
            "x": _w((lambda *s: _rng.normal(s) * 0.05)(B, S, D)),
            "Lambda_re": _w(Lambda_re),
            "Lambda_im": _w(Lambda_im),
            "B_re": _w(B_re),
            "B_im": _w(B_im),
            "C_re": _w(C_re),
            "C_im": _w(C_im),
            "log_dt": _w(log_dt),
            "Dskip": _w(Dskip),
        }
    _A_in = _A_setup()

    def _B_setup():
        B, S, D, F = 1, 2048, 512, 1376
        return {
            "x": _w((lambda *s: _rng.normal(s) * 0.05)(B, S, D)),
            "w_gate": _w((lambda *s: _rng.normal(s) * 0.05)(D, F)),
            "w_up": _w((lambda *s: _rng.normal(s) * 0.05)(D, F)),
            "w_down": _w((lambda *s: _rng.normal(s) * 0.05)(F, D)),
        }
    _B_in = _B_setup()

    return {
        "A_x": _A_in["x"],
        "A_Lambda_re": _A_in["Lambda_re"],
        "A_Lambda_im": _A_in["Lambda_im"],
        "A_B_re": _A_in["B_re"],
        "A_B_im": _A_in["B_im"],
        "A_C_re": _A_in["C_re"],
        "A_C_im": _A_in["C_im"],
        "A_log_dt": _A_in["log_dt"],
        "A_Dskip": _A_in["Dskip"],
        "B_x": _B_in["x"],
        "B_w_gate": _B_in["w_gate"],
        "B_w_up": _B_in["w_up"],
        "B_w_down": _B_in["w_down"],
    }

def reference(A_x, A_Lambda_re, A_Lambda_im, A_B_re, A_B_im, A_C_re, A_C_im, A_log_dt, A_Dskip, B_x, B_w_gate, B_w_up, B_w_down):
    def _A_ref(x, Lambda_re, Lambda_im, B_re, B_im, C_re, C_im, log_dt, Dskip):
        Bsz, L, H = x.shape
        Lam = Lambda_re + 1j * Lambda_im
        Bmat = B_re + 1j * B_im
        Cmat = C_re + 1j * C_im
        dt = jnp.exp(log_dt)
        Lam_bar = jnp.exp(dt * Lam)
        B_bar = ((Lam_bar - 1.0) / Lam)[:, None] * Bmat
        Bu = jnp.einsum("bld,pd->blp", x + 0j, B_bar)
        h = jnp.zeros_like(Bu[:, 0, :])
        hs = []
        for t in range(L):
            h = Lam_bar[None, :] * h + Bu[:, t, :]
            hs.append(h)
        hseq = jnp.stack(hs, 1)
        y = 2.0 * jnp.einsum("blp,dp->bld", hseq, Cmat).real + x * Dskip[None, None, :]
        return y

    def _B_ref(x, w_gate, w_up, w_down):
        return (_gelu(x @ w_gate) * (x @ w_up)) @ w_down

    x = A_x
    xn = _layernorm(x, axis=-1)
    return x + _A_ref(xn, A_Lambda_re, A_Lambda_im, A_B_re, A_B_im, A_C_re, A_C_im, A_log_dt, A_Dskip) + _B_ref(xn, B_w_gate, B_w_up, B_w_down)
```

```python
import functools
import numpy as np
import jax
import jax.numpy as jnp
from jax import lax
import jax.experimental.pallas as pl
import jax.experimental.pallas.tpu as pltpu

F32 = jnp.float32
BF16 = jnp.bfloat16
NT = (((1,), (1,)), ((), ()))


def _make(TM=512, FC=384, out_dtype=F32, vmem=110 * 1024 * 1024, ln_pos=2, NO=4, XS=4, scan_span=None):
    L, D, P, F = 2048, 512, 512, 1376
    NB = L // TM
    NC = P // 128
    S = TM + 4
    chunks = [(a, min(a + FC, F)) for a in range(0, F, FC)]
    NCH = len(chunks)
    OW = D // NO
    span = scan_span or max(1, NCH - 1)

    def kernel(x_hbm, lre_hbm, lim_hbm, bre_hbm, bim_hbm, cre_hbm, cim_hbm, ldt_hbm, dsk_hbm,
               wg_hbm, wu_hbm, wd_hbm, o_hbm,
               xbuf, v0, v1, v2, v3, bre, bim, cre, cim, wg, wu, wd, par_ref, u_ref, xnb_ref, base_ref, obuf,
               isem, osem):
        copies = []
        def mk(src, dst):
            c = pltpu.make_async_copy(src, dst, isem.at[len(copies)])
            copies.append(c)
            return c
        XR = TM // XS
        x0c = [mk(x_hbm.at[0, pl.ds(k * XR, XR), :], xbuf.at[pl.ds(k * XR, XR), :]) for k in range(XS)]
        vbuf = [v0, v1, v2, v3]
        vcopies = [mk(src, vbuf[k]) for k, src in enumerate((lre_hbm, lim_hbm, ldt_hbm, dsk_hbm))]
        bcopies = [mk(bre_hbm, bre), mk(bim_hbm, bim)]
        wcopies = []
        for (a, b) in chunks:
            wcopies.append([mk(src.at[pl.ds(a, b - a), :], dst.at[pl.ds(a, b - a), :])
                            for (src, dst) in ((wg_hbm, wg), (wu_hbm, wu), (wd_hbm, wd))])
        xc = [None] + [None] * (NB - 1)
        if NB > 1:
            xc[1] = mk(x_hbm.at[0, pl.ds(TM, TM), :], xbuf.at[pl.ds(TM, TM), :])
        ccopies = [mk(cre_hbm, cre), mk(cim_hbm, cim)]
        for i in range(2, NB):
            xc[i] = mk(x_hbm.at[0, pl.ds(i * TM, TM), :], xbuf.at[pl.ds(i * TM, TM), :])
        for c in copies:
            c.start()

        def ocopy(i, n):
            return pltpu.make_async_copy(obuf.at[pl.ds(i * TM, TM), pl.ds(n * OW, OW)],
                                         o_hbm.at[0, pl.ds(i * TM, TM), pl.ds(n * OW, OW)], osem.at[i * NO + n])

        def ln_rows(r0, nr, slot, dsk):
            x = xbuf[r0:r0 + nr, :].astype(F32)
            m = jnp.mean(x, axis=-1, keepdims=True)
            xc_ = x - m
            v = jnp.mean(xc_ * xc_, axis=-1, keepdims=True)
            xn = xc_ * lax.rsqrt(v + 1e-5)
            l0 = r0 % TM
            xnb_ref[slot, l0:l0 + nr, :] = xn.astype(BF16)
            base_ref[slot, l0:l0 + nr, :] = x + xn * dsk

        def prologue():
            for c in vcopies: c.wait()
            lre = v0[...].astype(F32).reshape(1, P)
            lim = v1[...].astype(F32).reshape(1, P)
            dt = jnp.exp(v2[...].astype(F32).reshape(1, P)).astype(BF16).astype(F32)
            mag = jnp.exp(dt * lre)
            ar = mag * jnp.cos(dt * lim)
            ai = mag * jnp.sin(dt * lim)
            den = lre * lre + lim * lim
            nr = ar - 1.0
            sr2 = 2.0 * (nr * lre + ai * lim) / den
            si2 = 2.0 * (ai * lre - nr * lim) / den
            a_r = jnp.concatenate([ar[:, c * 128:(c + 1) * 128] for c in range(NC)], axis=0)
            a_i = jnp.concatenate([ai[:, c * 128:(c + 1) * 128] for c in range(NC)], axis=0)
            a1 = jnp.concatenate([a_r, a_r], axis=0)
            a2 = jnp.concatenate([-a_i, a_i], axis=0)
            return sr2, si2, a1, a2

        def prologue_c(sr2, si2):
            for c in ccopies: c.wait()
            c_re = cre[...].astype(F32)
            c_im = cim[...].astype(F32)
            cre[...] = (c_re * sr2 - c_im * si2).astype(BF16)
            cim[...] = (-(c_re * si2) - c_im * sr2).astype(BF16)

        for c in vcopies[3:]: pass
        sr2, si2, a1, a2 = prologue()
        dsk = v3[...].astype(F32).reshape(1, D)
        for k in range(XS):
            x0c[k].wait()
            ln_rows(k * XR, XR, 0, dsk)

        st = {"h": jnp.zeros((8, 128), F32)}

        for i in range(NB):
            slot = i % 2
            first = i == 0
            xnb = xnb_ref[slot]
            if first: bcopies[0].wait()
            ur = lax.dot_general(xnb, bre[...], NT, preferred_element_type=F32)
            for c in range(NC):
                u_ref[pl.ds(c * S, TM), :] = ur[:, c * 128:(c + 1) * 128]
            if first: bcopies[1].wait()
            ui = lax.dot_general(xnb, bim[...], NT, preferred_element_type=F32)
            for c in range(NC):
                u_ref[pl.ds((NC + c) * S, TM), :] = ui[:, c * 128:(c + 1) * 128]

            def scan_cs(t0, t1):
                h = st["h"]
                for t in range(t0, t1):
                    ut = u_ref[pl.ds(t, 8, stride=S), :]
                    h = (a1 * h + ut) + a2 * pltpu.roll(h, 4, 0)
                    u_ref[pl.ds(t, 8, stride=S), :] = h
                st["h"] = h

            acc = None
            for j, (f0, f1) in enumerate(chunks):
                if first:
                    for c in wcopies[j]: c.wait()
                g = lax.dot_general(xnb, wg[f0:f1, :], NT, preferred_element_type=F32)
                u = lax.dot_general(xnb, wu[f0:f1, :], NT, preferred_element_type=F32)
                inner = g * (0.7978845608028654 + (0.7978845608028654 * 0.044715) * (g * g))
                a = (0.5 * g) * u * (1.0 + jnp.tanh(inner))
                if j < span:
                    scan_cs((j * TM) // span, ((j + 1) * TM) // span)
                if j == ln_pos and i + 1 < NB:
                    xc[i + 1].wait()
                    ln_rows((i + 1) * TM, TM, 1 - slot, dsk)
                d = jnp.dot(a.astype(BF16), wd[f0:f1, :], preferred_element_type=F32)
                acc = (base_ref[slot] + d) if acc is None else (acc + d)
            if first:
                prologue_c(sr2, si2)
            gr = jnp.concatenate([u_ref[pl.ds(c * S, TM), :] for c in range(NC)], axis=1).astype(BF16)
            gi = jnp.concatenate([u_ref[pl.ds((NC + c) * S, TM), :] for c in range(NC)], axis=1).astype(BF16)
            for n in range(NO):
                cs = slice(n * OW, (n + 1) * OW)
                y = acc[:, cs] + lax.dot_general(gr, cre[cs, :], NT, preferred_element_type=F32)
                y = y + lax.dot_general(gi, cim[cs, :], NT, preferred_element_type=F32)
                obuf[i * TM:(i + 1) * TM, cs] = y.astype(out_dtype)
                ocopy(i, n).start()
        for i in range(NB):
            for n in range(NO):
                ocopy(i, n).wait()

    def fn(A_x, A_Lambda_re, A_Lambda_im, A_B_re, A_B_im, A_C_re, A_C_im, A_log_dt, A_Dskip,
           B_x, B_w_gate, B_w_up, B_w_down):
        args = (A_x, A_Lambda_re, A_Lambda_im, A_B_re, A_B_im, A_C_re, A_C_im, A_log_dt, A_Dskip,
                B_w_gate.T, B_w_up.T, B_w_down)
        hbm = pl.BlockSpec(memory_space=pltpu.HBM)
        return pl.pallas_call(
            kernel,
            in_specs=[hbm] * len(args),
            out_specs=hbm,
            out_shape=jax.ShapeDtypeStruct(A_x.shape, out_dtype),
            scratch_shapes=[
                pltpu.VMEM((L, D), BF16),
                pltpu.VMEM((P,), BF16), pltpu.VMEM((P,), BF16), pltpu.VMEM((P,), BF16), pltpu.VMEM((D,), BF16),
                pltpu.VMEM((P, D), BF16), pltpu.VMEM((P, D), BF16),
                pltpu.VMEM((D, P), BF16), pltpu.VMEM((D, P), BF16),
                pltpu.VMEM((F, D), BF16), pltpu.VMEM((F, D), BF16), pltpu.VMEM((F, D), BF16),
                pltpu.VMEM((8, 128), F32),
                pltpu.VMEM((8 * S, 128), F32),
                pltpu.VMEM((2, TM, D), BF16),
                pltpu.VMEM((2, TM, D), F32),
                pltpu.VMEM((L, D), out_dtype),
                pltpu.SemaphoreType.DMA((XS + 4 + 2 + 3 * NCH + 2 + NB,)),
                pltpu.SemaphoreType.DMA((NB * NO,)),
            ],
            compiler_params=pltpu.CompilerParams(vmem_limit_bytes=vmem),
        )(*args)

    return fn


@jax.jit
def pallas_parallel_sum__ssm_conv_s5__geglu_ffn__prompt_kernel(
    A_x, A_Lambda_re, A_Lambda_im, A_B_re, A_B_im, A_C_re, A_C_im, A_log_dt, A_Dskip,
    B_x, B_w_gate, B_w_up, B_w_down,
):
    return _make()(A_x, A_Lambda_re, A_Lambda_im, A_B_re, A_B_im, A_C_re, A_C_im, A_log_dt, A_Dskip,
                   B_x, B_w_gate, B_w_up, B_w_down)
```

```python
import contextlib
import jax
import jax.numpy as jnp
from jax import lax
import jax.experimental.pallas as pl
import jax.experimental.pallas.tpu as pltpu

F32 = jnp.float32
BF16 = jnp.bfloat16
NT = (((1,), (1,)), ((), ()))
TN = (((0,), (0,)), ((), ()))


def dot_nt(a, b):
    return lax.dot_general(a, b, NT, preferred_element_type=F32)


def _make(TM=512, out_dtype=F32, vmem=110 * 1024 * 1024,
         bpieces=((0, 0, 256), (0, 256, 512), (1, 0, 512)),
         bwaits=((0,), (1,), (2,)),
         chunks0=((0, 256), (256, 640), (640, 1024), (1024, 1280), (1280, 1376)),
         wgroups=((0, 256), (256, 640), (640, 1280), (1280, 1376)),
         c_pos=None, c_wait=None, x_wait=None,
         chunksN=((0, 384), (384, 768), (768, 1280), (1280, 1376)),
         ln_pos0=4, ln_posN=2, NO=4, XS=4, span0=3, spanN=3, last_or=1,
         remT=False, scopes=False, wscopes=False, dmamode=0, ln_split=1, cproj_first=False, nobase=False, ln_piece=None, merge_last=False, head_piece=None):
    L, D, P, F = 2048, 512, 512, 1376
    NB = L // TM
    NC = P // 128
    S = TM + 4
    OW = D // NO
    NG = len(wgroups)
    FR = F % 128
    FM = F - FR
    c_pos = NG - 1 if c_pos is None else c_pos
    c_wait = NG - 1 if c_wait is None else c_wait
    x_wait = NG - 1 if x_wait is None else x_wait

    def kernel(x_hbm, lre_hbm, lim_hbm, bre_hbm, bim_hbm, cre_hbm, cim_hbm, ldt_hbm, dsk_hbm,
               wg_hbm, wu_hbm, wd_hbm, o_hbm,
               xbuf, v0, v1, v2, v3, bre, bim, cre, cim, wg, wu, wd, wrem, u_ref, xnb_ref, base_ref, obuf,
               isem, osem):
        copies = []

        class _W:
            def __init__(s_, c, n): s_.c = c; s_.n = n
            def start(s_):
                if dmamode != 2: s_.c.start()
            def wait(s_):
                if dmamode: return
                with (jax.named_scope(s_.n) if wscopes else contextlib.nullcontext()):
                    s_.c.wait()

        def mk(src, dst):
            c = _W(pltpu.make_async_copy(src, dst, isem.at[len(copies)]), f"w{len(copies):02d}")
            copies.append(c)
            return c

        vbuf = [v0, v1, v2, v3]
        vcopies = [mk(src, vbuf[k]) for k, src in enumerate((lre_hbm, lim_hbm, ldt_hbm, dsk_hbm))]
        XR = TM // XS
        x0c = [mk(x_hbm.at[0, pl.ds(k * XR, XR), :], xbuf.at[pl.ds(k * XR, XR), :]) for k in range(XS)]
        bcop = []
        for (which, n0, n1) in bpieces:
            src, dst = ((bre_hbm, bre), (bim_hbm, bim))[which]
            bcop.append(mk(src.at[pl.ds(n0, n1 - n0), :], dst.at[pl.ds(n0, n1 - n0), :]))
        wcop = []
        ccopies = None
        for gi_, (a, b) in enumerate(wgroups):
            if remT and a == FM:
                wcop.append([mk(wg_hbm.at[pl.ds(a, FR), :], wrem.at[pl.ds(0, FR), :]),
                             mk(wu_hbm.at[pl.ds(a, FR), :], wrem.at[pl.ds(FR, FR), :]),
                             mk(wd_hbm.at[pl.ds(a, FR), :], wd.at[pl.ds(a, FR), :])])
            else:
                wcop.append([mk(src.at[pl.ds(a, b - a), :], dst.at[pl.ds(a, b - a), :])
                             for (src, dst) in ((wg_hbm, wg), (wu_hbm, wu), (wd_hbm, wd))])
            if gi_ == c_pos:
                ccopies = [mk(cre_hbm, cre), mk(cim_hbm, cim)]
        xrest = [mk(x_hbm.at[0, pl.ds(i * TM, TM), :], xbuf.at[pl.ds(i * TM, TM), :]) for i in range(1, NB)]
        for c in copies:
            c.start()

        def nor(i, n):
            return last_or if (i == NB - 1 and n == NO - 1) else 1

        def ocopy(i, n, r):
            RO = TM // nor(i, n)
            rows = pl.ds(i * TM + r * RO, RO)
            return pltpu.make_async_copy(obuf.at[rows, pl.ds(n * OW, OW)],
                                         o_hbm.at[0, rows, pl.ds(n * OW, OW)], osem.at[i * NO + n + r])

        def ln_rows(r0, nr, slot, dsk):
            x = xbuf[r0:r0 + nr, :].astype(F32)
            m = jnp.mean(x, axis=-1, keepdims=True)
            xc_ = x - m
            v = jnp.mean(xc_ * xc_, axis=-1, keepdims=True)
            xn = xc_ * lax.rsqrt(v + 1e-5)
            l0 = r0 % TM
            xnb_ref[slot, l0:l0 + nr, :] = xn.astype(BF16)
            if not nobase:
                base_ref[slot, l0:l0 + nr, :] = x + xn * dsk

        def ln_rows_p(r0, nr, slot, dsk, piece):
            piece = piece or nr
            for q in range(0, nr, piece):
                ln_rows(r0 + q, piece, slot, dsk)

        def prologue():
            for c in vcopies: c.wait()
            lre = v0[...].astype(F32).reshape(1, P)
            lim = v1[...].astype(F32).reshape(1, P)
            dt = jnp.exp(v2[...].astype(F32).reshape(1, P)).astype(BF16).astype(F32)
            mag = jnp.exp(dt * lre)
            ar = mag * jnp.cos(dt * lim)
            ai = mag * jnp.sin(dt * lim)
            den = lre * lre + lim * lim
            nr = ar - 1.0
            sr2 = 2.0 * (nr * lre + ai * lim) / den
            si2 = 2.0 * (ai * lre - nr * lim) / den
            a_r = jnp.concatenate([ar[:, c * 128:(c + 1) * 128] for c in range(NC)], axis=0)
            a_i = jnp.concatenate([ai[:, c * 128:(c + 1) * 128] for c in range(NC)], axis=0)
            a1 = jnp.concatenate([a_r, a_r], axis=0)
            a2 = jnp.concatenate([-a_i, a_i], axis=0)
            return sr2, si2, a1, a2

        def prologue_c(sr2, si2):
            c_re = cre[...].astype(F32)
            c_im = cim[...].astype(F32)
            cre[...] = (c_re * sr2 - c_im * si2).astype(BF16)
            cim[...] = (-(c_re * si2) - c_im * sr2).astype(BF16)

        scope = jax.named_scope if scopes else (lambda n: contextlib.nullcontext())
        with scope("head"):
            sr2, si2, a1, a2 = prologue()
            dsk = v3[...].astype(F32).reshape(1, D)
            for k in range(XS):
                x0c[k].wait()
                if merge_last and k == XS - 1:
                    for w_ in bwaits[0]: bcop[w_].wait()
                ln_rows_p(k * XR, XR, 0, dsk, head_piece)

        st = {"h": jnp.zeros((8, 128), F32)}

        def scan_cs(t0, t1):
            h = st["h"]
            for t in range(t0, t1):
                ut = u_ref[pl.ds(t, 8, stride=S), :]
                h = (a1 * h + ut) + a2 * pltpu.roll(h, 4, 0)
                u_ref[pl.ds(t, 8, stride=S), :] = h
            st["h"] = h

        for i in range(NB):
          with scope(f"step{i}"):
            slot = i % 2
            first = i == 0
            xnb = xnb_ref[slot]
            pieces = bpieces if first else ((0, 0, P), (1, 0, P))
            for bi_, (which, n0, n1) in enumerate(pieces):
                if first and not (merge_last and bi_ == 0):
                    for w_ in bwaits[bi_]:
                        bcop[w_].wait()
                src = bre if which == 0 else bim
                uu = dot_nt(xnb, src[n0:n1, :])
                for c in range(n0 // 128, n1 // 128):
                    u_ref[pl.ds((which * NC + c) * S, TM), :] = uu[:, c * 128 - n0:(c + 1) * 128 - n0]

            chunks = chunks0 if first else chunksN
            span = span0 if first else spanN
            ln_pos = ln_pos0 if first else ln_posN
            acc = None
            for j, (f0, f1) in enumerate(chunks):
                if first:
                    for gi_, (a, b) in enumerate(wgroups):
                        if a == f0:
                            for c in wcop[gi_]: c.wait()
                            if gi_ == c_wait:
                                for c in ccopies: c.wait()
                            if gi_ == x_wait:
                                for c in xrest: c.wait()
                            if gi_ == c_wait:
                                prologue_c(sr2, si2)
                tr = remT and f0 == FM
                if tr:
                    gu = dot_nt(wrem[...], xnb)
                    g = gu[:FR]
                    u = gu[FR:]
                else:
                    g = dot_nt(xnb, wg[f0:f1, :])
                    u = dot_nt(xnb, wu[f0:f1, :])
                inner = g * (0.7978845608028654 + (0.7978845608028654 * 0.044715) * (g * g))
                a = (0.5 * g) * u * (1.0 + jnp.tanh(inner))
                if j < span:
                    scan_cs((j * TM) // span, ((j + 1) * TM) // span)
                if i + 1 < NB:
                    if ln_split == 1:
                        if j == ln_pos:
                            ln_rows_p((i + 1) * TM, TM, 1 - slot, dsk, ln_piece)
                    else:
                        for q in range(ln_split):
                            if j == min(ln_pos + q, len(chunks) - 1):
                                ln_rows_p((i + 1) * TM + q * (TM // ln_split), TM // ln_split, 1 - slot, dsk, ln_piece)
                if tr:
                    d = lax.dot_general(a.astype(BF16), wd[f0:f1, :], TN, preferred_element_type=F32)
                else:
                    d = jnp.dot(a.astype(BF16), wd[f0:f1, :], preferred_element_type=F32)
                if acc is None:
                    if nobase:
                        acc = (xbuf[i * TM:(i + 1) * TM, :].astype(F32) + xnb.astype(F32) * dsk) + d
                    else:
                        acc = base_ref[slot] + d
                else:
                    acc = acc + d
            gr = jnp.concatenate([u_ref[pl.ds(c * S, TM), :] for c in range(NC)], axis=1).astype(BF16)
            gi = jnp.concatenate([u_ref[pl.ds((NC + c) * S, TM), :] for c in range(NC)], axis=1).astype(BF16)
            for n in range(NO):
                cs = slice(n * OW, (n + 1) * OW)
                y = acc[:, cs] + dot_nt(gr, cre[cs, :])
                y = y + dot_nt(gi, cim[cs, :])
                obuf[i * TM:(i + 1) * TM, cs] = y.astype(out_dtype)
                for r in range(nor(i, n)):
                    ocopy(i, n, r).start()
        if dmamode == 1:
            for c in copies: c.c.wait()
        with scope("tail"):
            for i in range(NB):
                for n in range(NO):
                    for r in range(nor(i, n)):
                        ocopy(i, n, r).wait()

    def fn(A_x, A_Lambda_re, A_Lambda_im, A_B_re, A_B_im, A_C_re, A_C_im, A_log_dt, A_Dskip,
           B_x, B_w_gate, B_w_up, B_w_down):
        args = (A_x, A_Lambda_re, A_Lambda_im, A_B_re, A_B_im, A_C_re, A_C_im, A_log_dt, A_Dskip,
                B_w_gate.T, B_w_up.T, B_w_down)
        hbm = pl.BlockSpec(memory_space=pltpu.HBM)
        return pl.pallas_call(
            kernel,
            in_specs=[hbm] * len(args),
            out_specs=hbm,
            out_shape=jax.ShapeDtypeStruct(A_x.shape, out_dtype),
            scratch_shapes=[
                pltpu.VMEM((L, D), BF16),
                pltpu.VMEM((P,), BF16), pltpu.VMEM((P,), BF16), pltpu.VMEM((P,), BF16), pltpu.VMEM((D,), BF16),
                pltpu.VMEM((P, D), BF16), pltpu.VMEM((P, D), BF16),
                pltpu.VMEM((D, P), BF16), pltpu.VMEM((D, P), BF16),
                pltpu.VMEM((F, D), BF16), pltpu.VMEM((F, D), BF16), pltpu.VMEM((F, D), BF16),
                pltpu.VMEM((2 * FR, D), BF16),
                pltpu.VMEM((8 * S, 128), F32),
                pltpu.VMEM((2, TM, D), BF16),
                pltpu.VMEM((2, TM, D), F32),
                pltpu.VMEM((L, D), out_dtype),
                pltpu.SemaphoreType.DMA((XS + 4 + len(bpieces) + 3 * NG + 2 + NB - 1,)),
                pltpu.SemaphoreType.DMA((NB * NO + last_or - 1,)),
            ],
            compiler_params=pltpu.CompilerParams(vmem_limit_bytes=vmem),
        )(*args)

    return fn


@jax.jit
def pallas_parallel_sum__ssm_conv_s5__geglu_ffn__prompt_kernel(
    A_x, A_Lambda_re, A_Lambda_im, A_B_re, A_B_im, A_C_re, A_C_im, A_log_dt, A_Dskip,
    B_x, B_w_gate, B_w_up, B_w_down,
):
    return _make(remT=True, nobase=True, merge_last=True, bpieces=((0,0,128),(0,128,512),(1,0,512)), bwaits=((0,),(1,),(2,)))(A_x, A_Lambda_re, A_Lambda_im, A_B_re, A_B_im, A_C_re, A_C_im, A_log_dt, A_Dskip,
                   B_x, B_w_gate, B_w_up, B_w_down)
```

```python
import jax
import jax.numpy as jnp
from jax import lax
import jax.experimental.pallas as pl
import jax.experimental.pallas.tpu as pltpu

_F32 = jnp.float32
_BF16 = jnp.bfloat16
_NT = (((1,), (1,)), ((), ()))
_TN = (((0,), (0,)), ((), ()))
_LANES = 128

_TM = 512
_XS = 4
_NO = 4
_LAST_SPLIT = 16
_NSEM = 8
_GELU_C0 = 0.7978845608028654
_GELU_C1 = 0.7978845608028654 * 0.044715


def _dot_nt(a, b):
    return lax.dot_general(a, b, _NT, preferred_element_type=_F32)


def _build(L, D, P, F):
    TM, XS, NO, NS = _TM, _XS, _NO, _NSEM
    NB = L // TM
    NC = P // _LANES
    S = TM + 4
    OW = D // NO
    FR = F % _LANES
    FM = F - FR
    XR = TM // XS
    assert L % TM == 0 and P == 4 * _LANES and D == NO * _LANES and FR % 16 == 0 and FR > 0

    b_pieces = ((0, 0, 128), (0, 128, 256), (0, 256, P), (1, 0, 256), (1, 256, P))
    chunks = ((0, 384), (384, 768), (768, FM), (FM, F))
    scan_span = 3

    O_B = 0
    O_G = O_B + 2 * P
    O_U = O_G + FM
    O_R = O_U + FM
    O_D = O_R + 2 * FR
    O_C = O_D + F
    O_A = O_C + 2 * D
    R = O_A + 16

    def kernel(x_hbm, lre_hbm, lim_hbm, bre_hbm, bim_hbm, cre_hbm, cim_hbm, ldt_hbm, dsk_hbm,
               wg_hbm, wu_hbm, wd_hbm, o_hbm,
               xbuf, lre_v, lim_v, ldt_v, dsk_v, wall, u_ref, xn_ref, obuf, sem):
        x2 = x_hbm.at[0]

        def wrows(src, a, b, off):
            return (src.at[pl.ds(a, b - a), :], wall.at[pl.ds(off, b - a), :])

        def w_gate(a, b):
            return wrows(wg_hbm, a, b, O_R if a == FM else O_G + a)

        def w_up(a, b):
            return wrows(wu_hbm, a, b, O_R + FR if a == FM else O_U + a)

        def w_down(a, b):
            return wrows(wd_hbm, a, b, O_D + a)

        groups = [("vec", [(lre_hbm, lre_v), (lim_hbm, lim_v), (ldt_hbm, ldt_v), (dsk_hbm, dsk_v)])]
        for k in range(XS):
            groups.append((f"x{k}", [(x2.at[pl.ds(k * XR, XR), :], xbuf.at[pl.ds(k * XR, XR), :])]))
        for k, (which, n0, n1) in enumerate(b_pieces):
            groups.append((f"b{k}", [wrows((bre_hbm, bim_hbm)[which], n0, n1, O_B + which * P + n0)]))
        groups.append(("g0", [w_gate(*chunks[0])]))
        groups.append(("u0", [w_up(*chunks[0])]))
        groups.append(("d0", [w_down(*chunks[0])]))
        groups.append(("w1", [w_gate(*chunks[1]), w_up(*chunks[1]), w_down(*chunks[1])]))
        groups.append(("w2", [f(*c) for c in chunks[2:] for f in (w_gate, w_up, w_down)]))
        groups.append(("c", [wrows(cre_hbm, 0, D, O_C), wrows(cim_hbm, 0, D, O_C + D),
                             (x2.at[pl.ds(TM, L - TM), :], xbuf.at[pl.ds(TM, L - TM), :])]))
        index = {name: k for k, (name, _) in enumerate(groups)}

        def copies(k):
            return [pltpu.make_async_copy(s_, d_, sem.at[k % NS]) for s_, d_ in groups[k][1]]

        started = [0]

        def start_upto(k):
            while started[0] < min(k, len(groups)):
                for c in copies(started[0]):
                    c.start()
                started[0] += 1

        def wait(name):
            k = index[name]
            assert k < started[0]
            for c in copies(k):
                c.wait()
            start_upto(k + 1 + NS)

        start_upto(NS)
        out_sem = sem.at[len(groups) % NS]

        wait("vec")
        lre = lre_v[...].astype(_F32).reshape(1, P)
        lim = lim_v[...].astype(_F32).reshape(1, P)
        dt = jnp.exp(ldt_v[...].astype(_F32).reshape(1, P)).astype(_BF16).astype(_F32)
        mag = jnp.exp(dt * lre)
        ar = mag * jnp.cos(dt * lim)
        ai = mag * jnp.sin(dt * lim)
        den = lre * lre + lim * lim
        nr = ar - 1.0
        sr = 2.0 * (nr * lre + ai * lim) / den
        si = 2.0 * (ai * lre - nr * lim) / den

        def fold(v):
            return jnp.concatenate([v[:, c * _LANES:(c + 1) * _LANES] for c in range(NC)], axis=0)

        a_r, a_i, s_r, s_i = fold(ar), fold(ai), fold(sr), fold(si)
        a1 = jnp.concatenate([a_r, a_r], axis=0)
        a2 = jnp.concatenate([-a_i, a_i], axis=0)
        s1 = jnp.concatenate([s_r, -s_r], axis=0)
        s2 = jnp.concatenate([-s_i, -s_i], axis=0)
        dskip = dsk_v[...].astype(_F32).reshape(1, D)

        def layernorm_rows(r0, nrows, slot):
            x = xbuf[r0:r0 + nrows, :].astype(_F32)
            m = jnp.mean(x, axis=-1, keepdims=True)
            xc = x - m
            v = jnp.mean(xc * xc, axis=-1, keepdims=True)
            l0 = r0 % TM
            xn_ref[slot, l0:l0 + nrows, :] = (xc * lax.rsqrt(v + 1e-5)).astype(_BF16)

        for k in range(XS):
            wait(f"x{k}")
            layernorm_rows(k * XR, XR, 0)

        state = {"h": jnp.zeros((8, _LANES), _F32), "r": jnp.zeros((8, _LANES), _F32)}

        def scan(t0, t1):
            h, r = state["h"], state["r"]
            for t in range(t0, t1):
                row = pl.ds(t, 8, stride=S)
                h = (a1 * h + u_ref[row, :]) + a2 * r
                r = pltpu.roll(h, 4, 0)
                u_ref[row, :] = s1 * h + s2 * r
            state["h"], state["r"] = h, r

        for i in range(NB):
            first = i == 0
            slot = i % 2

            for k, (which, n0, n1) in enumerate(b_pieces if first else ((0, 0, P), (1, 0, P))):
                if first:
                    wait(f"b{k}")
                o = O_B + which * P
                u = _dot_nt(xn_ref[slot], wall[o + n0:o + n1, :])
                for c in range(n0 // _LANES, n1 // _LANES):
                    u_ref[pl.ds((which * NC + c) * S, TM), :] = u[:, c * _LANES - n0:(c + 1) * _LANES - n0]
                if first and k + 1 < len(b_pieces):
                    wall[O_A:O_A + 16, 0:_LANES] = u[TM // 2:TM // 2 + 16, n1 - n0 - _LANES:].astype(_BF16)

            acc = None
            for j, (f0, f1) in enumerate(chunks):
                remainder = f0 == FM
                if first:
                    if j == 0:
                        wait("g0")
                    elif j < 3:
                        wait(f"w{j}")
                    if remainder:
                        wait("c")
                if remainder:
                    gu = _dot_nt(wall[O_R:O_R + 2 * FR, :], xn_ref[slot])
                    g, up = gu[:FR], gu[FR:]
                else:
                    g = _dot_nt(xn_ref[slot], wall[O_G + f0:O_G + f1, :])
                    if first and j == 0:
                        wait("u0")
                    up = _dot_nt(xn_ref[slot], wall[O_U + f0:O_U + f1, :])
                act = (0.5 * g) * up * (1.0 + jnp.tanh(g * (_GELU_C0 + _GELU_C1 * (g * g))))
                if j < scan_span:
                    scan((j * TM) // scan_span, ((j + 1) * TM) // scan_span)
                if i + 1 < NB and j == (3 if first else 2):
                    layernorm_rows((i + 1) * TM, TM, 1 - slot)
                if first and j == 0:
                    wait("d0")
                wd = wall[O_D + f0:O_D + f1, :]
                if remainder:
                    d = lax.dot_general(act.astype(_BF16), wd, _TN, preferred_element_type=_F32)
                else:
                    d = jnp.dot(act.astype(_BF16), wd, preferred_element_type=_F32)
                if acc is None:
                    acc = (xbuf[i * TM:(i + 1) * TM, :].astype(_F32) + xn_ref[slot].astype(_F32) * dskip) + d
                else:
                    acc = acc + d

            h_re = jnp.concatenate([u_ref[pl.ds(c * S, TM), :] for c in range(NC)], axis=1).astype(_BF16)
            h_im = jnp.concatenate([u_ref[pl.ds((NC + c) * S, TM), :] for c in range(NC)], axis=1).astype(_BF16)
            for n in range(NO):
                cols = slice(n * OW, (n + 1) * OW)
                y = acc[:, cols] + _dot_nt(h_re, wall[O_C + n * OW:O_C + (n + 1) * OW, :])
                y = y + _dot_nt(h_im, wall[O_C + D + n * OW:O_C + D + (n + 1) * OW, :])
                split = _LAST_SPLIT if (i == NB - 1 and n == NO - 1) else 1
                nrows = TM // split
                for q in range(split):
                    r0 = i * TM + q * nrows
                    obuf[r0:r0 + nrows, cols] = y[q * nrows:(q + 1) * nrows]
                    pltpu.make_async_copy(obuf.at[pl.ds(r0, nrows), pl.ds(n * OW, OW)],
                                          o_hbm.at[0, pl.ds(r0, nrows), pl.ds(n * OW, OW)], out_sem).start()

        pltpu.make_async_copy(obuf, o_hbm.at[0], out_sem).wait()

    scratch = [
        pltpu.VMEM((L, D), _BF16),
        pltpu.VMEM((P,), _BF16), pltpu.VMEM((P,), _BF16),
        pltpu.VMEM((P,), _BF16), pltpu.VMEM((D,), _BF16),
        pltpu.VMEM((R, D), _BF16),
        pltpu.VMEM((2 * NC * S, _LANES), _F32),
        pltpu.VMEM((2, TM, D), _BF16),
        pltpu.VMEM((L, D), _F32),
        pltpu.SemaphoreType.DMA((NS,)),
    ]
    return kernel, scratch


@jax.jit
def pallas_parallel_sum__ssm_conv_s5__geglu_ffn__prompt_kernel(
    A_x: jax.Array,
    A_Lambda_re: jax.Array,
    A_Lambda_im: jax.Array,
    A_B_re: jax.Array,
    A_B_im: jax.Array,
    A_C_re: jax.Array,
    A_C_im: jax.Array,
    A_log_dt: jax.Array,
    A_Dskip: jax.Array,
    B_x: jax.Array,
    B_w_gate: jax.Array,
    B_w_up: jax.Array,
    B_w_down: jax.Array,
):
    del B_x
    _, L, D = A_x.shape
    P = A_B_re.shape[0]
    F = B_w_gate.shape[1]
    kernel, scratch = _build(L, D, P, F)
    args = (A_x, A_Lambda_re, A_Lambda_im, A_B_re, A_B_im, A_C_re, A_C_im, A_log_dt, A_Dskip,
            B_w_gate.T, B_w_up.T, B_w_down)
    hbm = pl.BlockSpec(memory_space=pltpu.HBM)
    return pl.pallas_call(
        kernel,
        in_specs=[hbm] * len(args),
        out_specs=hbm,
        out_shape=jax.ShapeDtypeStruct(A_x.shape, _F32),
        scratch_shapes=scratch,
        compiler_params=pltpu.CompilerParams(
            vmem_limit_bytes=64 * 1024 * 1024,
            flags={"XLA_TPU_RESCHEDULE_DMA_DONES": True},
        ),
    )(*args)
```
